```python
import os as _os
_os.environ.setdefault("JAX_PLATFORMS", "cpu")
import jax
import jax.numpy as jnp

def _softmax(x, axis=-1):
    return jax.nn.softmax(x, axis=axis)
def _gelu(x):
    return jax.nn.gelu(x, approximate=True)
def _silu(x):
    return jax.nn.silu(x)
def _sigmoid(x):
    return jax.nn.sigmoid(x)
def _layernorm(x, axis=-1, eps=1e-5):
    m = jnp.mean(x, axis=axis, keepdims=True)
    v = jnp.var(x, axis=axis, keepdims=True)
    return (x - m) / jnp.sqrt(v + eps)
def _scatter_add(tgt, idx, src, axis=0):
    return tgt.at[idx].add(src)
def _segment_sum(src, seg, n):
    return jax.ops.segment_sum(src, seg, n)
class _Rng:
    def __init__(self, key):
        self._k = key
    def _next(self):
        self._k, sub = jax.random.split(self._k)
        return sub
    def normal(self, shape):
        return jax.random.normal(self._next(), shape, dtype=jnp.bfloat16)
    def randint(self, lo, hi, shape):
        return jax.random.randint(self._next(), shape, lo, hi, dtype=jnp.int32)
    def uniform(self, shape, lo=0.0, hi=1.0):
        return jax.random.uniform(self._next(), shape, jnp.bfloat16, lo, hi)
    def permutation(self, n):
        return jax.random.permutation(self._next(), n)


kernel_name = 'interleave_layers__sliding_local_dilated__mixer_channel_mlp__prompt'

def setup_inputs():
    _rng = _Rng(jax.random.key(int.from_bytes(__import__("os").urandom(4), "little")))
    _w = (lambda a: (lambda t: t.astype(jnp.bfloat16) if jnp.issubdtype(t.dtype, jnp.floating) else t)(jnp.asarray(a)))
    def _A_setup():
        B, S, D = 1, 2048, 512
        return {
            "x": _w((lambda *s: _rng.normal(s) * 0.05)(B, S, D)),
            "wqkv": _w((lambda *s: _rng.normal(s) * 0.05)(D, 3 * D)),
            "wo": _w((lambda *s: _rng.normal(s) * 0.05)(D, D)),
        }
    _A_in = _A_setup()

    def _B_setup():
        B, S, D, F = 1, 2048, 512, 1376
        return {
            "x": _w((lambda *s: _rng.normal(s) * 0.05)(B, S, D)),
            "w1": _w((lambda *s: _rng.normal(s) * 0.4)(D, F) * (D ** -0.5)),
            "b1": _w((lambda *s: _rng.normal(s) * 0.4)(F)),
            "w2": _w((lambda *s: _rng.normal(s) * 0.4)(F, D) * (F ** -0.5)),
            "b2": _w((lambda *s: _rng.normal(s) * 0.4)(D)),
        }
    _B_in = _B_setup()

    return {
        "A_x": _A_in["x"],
        "A_wqkv": _A_in["wqkv"],
        "A_wo": _A_in["wo"],
        "B_x": _B_in["x"],
        "B_w1": _B_in["w1"],
        "B_b1": _B_in["b1"],
        "B_w2": _B_in["w2"],
        "B_b2": _B_in["b2"],
    }

def reference(A_x, A_wqkv, A_wo, B_x, B_w1, B_b1, B_w2, B_b2):
    def _A_ref(x, wqkv, wo):
        B, S, D = x.shape
        H = 32; Dh = D // H
        W, dil = 8, 2
        qkv = (lambda x, *d: x.transpose(*d))((x @ wqkv).reshape(B, S, 3, H, Dh), 2, 0, 3, 1, 4)
        q, k, v = qkv[0], qkv[1], qkv[2]
        scale = Dh ** -0.5
        pos = jnp.arange(S)
        off = jnp.arange(W) * dil
        idx = pos[:, None] - off[None, :]
        mask = idx >= 0
        idx_c = jnp.where(mask, idx, 0).reshape(-1)
        kg = k[:, :, idx_c, :].reshape(B, H, S, W, Dh)
        vg = v[:, :, idx_c, :].reshape(B, H, S, W, Dh)
        logits = jnp.einsum("bhsd,bhswd->bhsw", q, kg) * scale
        logits = jnp.where(mask[None, None, :, :], logits, -1e9)
        attn = _softmax(logits, axis=-1)
        o = jnp.einsum("bhsw,bhswd->bhsd", attn, vg)
        return (lambda x, *d: x.transpose(*d))(o, 0, 2, 1, 3).reshape(B, S, D) @ wo

    def _B_ref(x, w1, b1, w2, b2):
        y = _layernorm(x, axis=-1)
        h = _gelu(jnp.einsum("bsd,df->bsf", y, w1) + b1)
        return jnp.einsum("bsf,fd->bsd", h, w2) + b2

    x = A_x
    x = x + _A_ref(_layernorm(x, axis=-1), A_wqkv, A_wo)
    x = x + _B_ref(_layernorm(x, axis=-1), B_w1, B_b1, B_w2, B_b2)
    x = x + _A_ref(_layernorm(x, axis=-1), A_wqkv, A_wo)
    x = x + _B_ref(_layernorm(x, axis=-1), B_w1, B_b1, B_w2, B_b2)
    return x
```

```python
import functools
import math
import os
import jax
import jax.numpy as jnp
from jax import lax
import jax.experimental.pallas as pl
import jax.experimental.pallas.tpu as pltpu

S, D, F = 2048, 512, 1376
H, DH, W, DIL = 32, 16, 8, 2
EPS = 1e-5
HALO = int(os.environ.get('HALO', 64))
HUSE = 16
T = 256
TH = T // 2
R = int(os.environ.get('R', 8))
NL = D // 128
NT = S // T
NITEMS = 2 * NT
NSTEPS = NITEMS // 2 + 1
NSPLIT = int(os.environ.get('NSPLIT', 384))
CHAIN = int(os.environ.get('CHAIN', 3))
TOKEN = int(os.environ.get('TOKEN', 9))
HK0 = int(os.environ.get('HK0', 160))
HKL = int(os.environ.get('HKL', 168))
QS = int(os.environ.get('QS', 256))
CHAIN0 = int(os.environ.get('CHAIN0', 3))
CHAINL = int(os.environ.get('CHAINL', 3))

F32 = jnp.float32
BF16 = jnp.bfloat16
U32 = jnp.uint32
NT_DIMS = (((1,), (1,)), ((), ()))
LOG2E = math.log2(math.e)

SEM_X0, SEM_WQ, SEM_WK, SEM_G3, SEM_W1, SEM_LATE, SEM_OUT = range(7)
NSEM = 7


def _pk(x):
    return pltpu.bitcast(x, U32)


def _upk(x):
    return pltpu.bitcast(x, BF16)


def _ln(x):
    m = jnp.mean(x, axis=-1, keepdims=True)
    xc = x - m
    v = jnp.mean(xc * xc, axis=-1, keepdims=True)
    return xc * lax.rsqrt(v + EPS)


def _ln2(x):
    m = jnp.mean(x, axis=-1, keepdims=True)
    xc = x - m
    v = jnp.mean(xc * xc, axis=-1, keepdims=True)
    return xc * lax.rsqrt(v * (1.0 + EPS) + EPS * EPS)


def _gelu(x):
    c0 = math.sqrt(2.0 / math.pi)
    c1 = c0 * 0.044715
    u = x * (c0 + c1 * (x * x))
    hx = 0.5 * x
    return hx + hx * jnp.tanh(u)


def _perm_matrix():
    r = lax.broadcasted_iota(jnp.int32, (128, 128), 0)
    c = lax.broadcasted_iota(jnp.int32, (128, 128), 1)
    return (((r % 8) * DH + (r // 8)) == c).astype(BF16)


def _interleave(parts):
    rows = []
    for d in range(DH):
        for J in range(NL):
            rows.append(parts[J][d * 8:(d + 1) * 8, :])
    return jnp.concatenate(rows, axis=0).astype(BF16)


def _kernel(x_hbm, wqkv_hbm, wo_hbm, w1t_hbm, b1_hbm, w2_hbm, b2_hbm, out_hbm,
            xe, xo, wqkv_raw, wo_raw, w1t_s, w2_s, b1_s, b2_s, wqkvt_p, wo_p,
            qa, ka, va, qb, kb, vb, x1a, x1b, g_s, xn0_s, xn1_s, o_s, sems):
    step = pl.program_id(0)
    xbuf = (xe, xo)
    qs, ks, vs, x1s = (qa, qb), (ka, kb), (va, vb), (x1a, x1b)

    def rows_at(slot, r0, n):
        if isinstance(slot, int):
            return pl.ds(slot * T + r0, n)
        return pl.ds(pl.multiple_of(slot * T + r0, TH), n)

    def x_in_copy(t):
        return pltpu.make_async_copy(
            x_hbm.at[0, pl.ds(t * T, T), :], xbuf[t % 2].at[pl.ds((t // 2) * T, T), :], sems.at[SEM_X0 if t == 0 else (SEM_G3 if t == 1 else SEM_LATE)])

    def x_out_copy(par, slot, r0=0, n=T, sem_off=0):
        return pltpu.make_async_copy(
            xbuf[par].at[rows_at(slot, r0, n), :],
            out_hbm.at[0, rows_at(2 * slot + par, r0, n), :],
            sems.at[SEM_OUT])

    def wqkv_copy(b):
        return pltpu.make_async_copy(
            wqkv_hbm.at[:, pl.ds(b * D, D)], wqkv_raw.at[b], sems.at[(SEM_WQ, SEM_WK, SEM_G3)[b]])

    def wo_copy():
        return pltpu.make_async_copy(wo_hbm, wo_raw, sems.at[SEM_G3])

    def w1_copies():
        cps = [pltpu.make_async_copy(w1t_hbm.at[:, pl.ds(j * 128, 128)], w1t_s.at[j], sems.at[SEM_W1])
               for j in range(NL)]
        cps += [pltpu.make_async_copy(b1_hbm, b1_s, sems.at[SEM_W1])]
        return cps

    def late_copies():
        cps = [pltpu.make_async_copy(w2_hbm.at[:, pl.ds(j * 128, 128)], w2_s.at[j], sems.at[SEM_LATE])
               for j in range(NL)]
        cps += [pltpu.make_async_copy(b2_hbm, b2_s, sems.at[SEM_LATE])]
        cps += [x_in_copy(t) for t in range(2, NT)]
        return cps

    def wcols(ref, j0, j1):
        return jnp.concatenate([_upk(ref.at[j].bitcast(U32)[...]) for j in range(j0, j1)], axis=1)

    def load_x(par, slot, r0=0, n=T):
        return xbuf[par][rows_at(slot, r0, n), :].astype(F32)

    def proj(xn, par, c0, c1):
        qscale = (DH ** -0.5) * LOG2E
        res = lax.dot_general(xn, _upk(wqkvt_p[c0 // 2:c1 // 2, :]), NT_DIMS, preferred_element_type=F32)
        for c in range(c0, c1, 128):
            blk = res[:, c - c0:c - c0 + 128]
            b, j = c // D, (c % D) // 128
            if b == 0:
                qs[par][0:T, j * 128:(j + 1) * 128] = blk * qscale
            elif b == 1:
                ks[par][j, HALO:HALO + T, :] = blk
            else:
                vs[par][j, HALO:HALO + T, :] = blk

    def halo_copy(par):
        for j in range(NL):
            ks[par][j, HALO - HUSE:HALO, :] = ks[1 - par][j, HALO + T - HUSE:HALO + T, :]
            vs[par][j, HALO - HUSE:HALO, :] = vs[1 - par][j, HALO + T - HUSE:HALO + T, :]

    def zoff(k):
        return pl.multiple_of(lax.shift_right_logical(step, k) * 8, 8)

    def attention(par, row0, chain, ra=0, rb=T, hooks=None):
        q_s, k_s, v_s = qs[par], ks[par], vs[par]
        chunks = list(range(ra // R, rb // R))
        z1, z2 = zoff(10), zoff(11)

        def load_q(c):
            qq = q_s[pl.ds(z1 + c * R, R), :]
            return [qq[:, j * 128:(j + 1) * 128] for j in range(NL)]

        pend = {}
        for c in chunks[:chain]:
            pend[c] = load_q(c)
        for c in chunks:
            r0 = c * R
            q = pend.pop(c)
            logits = []
            for w in range(W):
                st = HALO + r0 - DIL * w
                acc = None
                for j in range(NL):
                    p = q[j] * k_s[j, st:st + R, :]
                    acc = p if acc is None else acc + p
                acc = acc + pltpu.roll(acc, 64, 1)
                acc = acc + pltpu.roll(acc, 32, 1)
                if r0 < DIL * w:
                    row = lax.broadcasted_iota(jnp.int32, (R, 128), 0) + (row0 + r0)
                    acc = jnp.where(row >= DIL * w, acc, -1e9 * LOG2E)
                logits.append(acc)
            m = logits[0]
            for w in range(1, W):
                m = jnp.maximum(m, logits[w])
            ps = [jnp.exp2(lg - m) for lg in logits]
            den = ps[0]
            for w in range(1, W):
                den = den + ps[w]
            inv = pl.reciprocal(den, approx=True)
            outs = []
            for j in range(NL):
                acc = None
                for w in range(W):
                    st = HALO + r0 - DIL * w
                    t = ps[w] * v_s[j, st:st + R, :]
                    acc = t if acc is None else acc + t
                outs.append(acc * inv)
            o_s[r0:r0 + R, :] = jnp.concatenate(outs, axis=1)
            q_s[pl.ds(z2 + T, 8), 0:128] = outs[NL - 1][0:8, :]
            if c + chain <= chunks[-1]:
                pend[c + chain] = load_q(c + chain)
            if hooks and (r0 + R) in hooks:
                hooks[r0 + R](outs[NL - 1][0:8, :])

    def w2_part(par, slot, c0, c1, r0=0, n=T, g=None):
        if g is None:
            g = _upk(g_s[r0 // 2:(r0 + n) // 2, :])
        b2 = b2_s[...].astype(F32)[None, :]
        acc = jnp.dot(g, wcols(w2_s, c0 // 128, c1 // 128), preferred_element_type=F32)
        x2 = x1s[par][r0:r0 + n, c0:c1] + (acc + b2[:, c0:c1])
        xbuf[par][rows_at(slot, r0, n), c0:c1] = x2.astype(BF16)

    def wo_mm(par, slot, r0=0, n=T):
        o = o_s[r0:r0 + n, :].astype(BF16)
        x1 = load_x(par, slot, r0, n) + jnp.dot(o, _upk(wo_p[...]), preferred_element_type=F32)
        x1s[par][r0:r0 + n, :] = x1
        return x1

    def ln2_after(par, r0, n, tok):
        x1s[par][pl.ds(zoff(11) + T, 8), 0:128] = tok
        return _ln2(x1s[par][pl.ds(zoff(10) + r0, n), :]).astype(BF16)

    def wo_ln2(par, slot, r0=0, n=T):
        return _ln2(wo_mm(par, slot, r0, n)).astype(BF16)

    def w1_gelu(y, r0=0, n=T):
        b1 = b1_s[...].astype(F32)[None, :]
        h = lax.dot_general(y, wcols(w1t_s, 0, NL), NT_DIMS, preferred_element_type=F32) + b1
        gl = _gelu(h)
        g_s[r0 // 2:(r0 + n) // 2, :] = _pk(gl.astype(BF16))
        return gl

    def body(sig, par, chain, token=None):
        slot_b = (sig % NT) // 2
        slot_c = ((sig + NT - 1) % NT) // 2
        slot_a = ((sig + 1) % NT) // 2
        xa = load_x(1 - par, slot_a)
        g = _upk(g_s[...])
        w2_part(1 - par, slot_c, 0, NSPLIT, g=g)
        proj(_ln(xa).astype(BF16), 1 - par, 0, 3 * D)
        halo_copy(1 - par)
        attention(par, (sig % NT) * T, chain)
        y = wo_ln2(par, slot_b)
        w2_part(1 - par, slot_c, NSPLIT, D, g=g)
        gl = w1_gelu(y)
        if token is not None:
            qs[1 - par][pl.ds(zoff(11) + T, 8), 0:128] = gl[T - 8:T, token * 128:(token + 1) * 128]

    def prep_qkv(b, Pi):
        parts = [lax.dot_general(Pi, wqkv_raw[b, :, J * 128:(J + 1) * 128], NT_DIMS, preferred_element_type=F32)
                 for J in range(NL)]
        wqkvt_p[b * D // 2:(b + 1) * D // 2, :] = _pk(_interleave(parts))

    @pl.when(step == 0)
    def _first():
        x_in_copy(0).start()
        wqkv_copy(0).start()
        wqkv_copy(1).start()
        z = jnp.zeros((HUSE, 128), F32)
        for j in range(NL):
            ka[j, HALO - HUSE:HALO, :] = z
            va[j, HALO - HUSE:HALO, :] = z
        Pi = _perm_matrix()
        x_in_copy(0).wait()
        wqkv_copy(2).start()
        x_in_copy(1).start()
        wo_copy().start()
        xn0_s[...] = _pk(_ln(load_x(0, 0)).astype(BF16))
        wqkv_copy(0).wait()
        prep_qkv(0, Pi)
        proj(_upk(xn0_s[...]), 0, 0, QS)
        wqkv_copy(1).wait()
        for c in w1_copies():
            c.start()
        prep_qkv(1, Pi)
        proj(_upk(xn0_s[...]), 0, QS, 2 * D)
        wqkv_copy(2).wait()
        x_in_copy(1).wait()
        wo_copy().wait()
        for c in late_copies():
            c.start()
        prep_qkv(2, Pi)
        parts = [jnp.dot(Pi, wo_raw[J * 128:(J + 1) * 128, :], preferred_element_type=F32) for J in range(NL)]
        wo_p[...] = _pk(_interleave(parts))
        proj(_upk(xn0_s[...]), 0, 2 * D, 3 * D)
        xn1 = _ln(load_x(1, 0)).astype(BF16)
        xn1_s[...] = _pk(xn1)
        proj(xn1, 1, 0, 2 * D)
        attention(0, 0, CHAIN0, 0, TH)
        for c in w1_copies():
            c.wait()
        x1h = wo_mm(0, 0, 0, TH)
        ys = []
        attention(0, 0, CHAIN0, TH, T, hooks={HK0: lambda tok: ys.append(ln2_after(0, 0, TH, tok))})
        ya = ys[0]
        proj(_upk(xn1_s[...]), 1, 2 * D, 2 * D + 256)
        w1_gelu(ya, 0, TH)
        yb = wo_ln2(0, 0, TH, TH)
        proj(_upk(xn1_s[...]), 1, 2 * D + 256, 3 * D)
        halo_copy(1)
        w1_gelu(yb, TH, TH)
        for c in late_copies():
            c.wait()

    @pl.when(jnp.logical_and(step > 0, step < NSTEPS - 1))
    def _mid():
        body(2 * step - 1, 1, CHAIN, token=TOKEN)
        body(2 * step, 0, CHAIN)

        @pl.when(step >= NT // 2 + 1)
        def _():
            slot = step - (NT // 2 + 1)
            x_out_copy(0, slot).start()
            x_out_copy(1, slot).start()

    @pl.when(step == NSTEPS - 1)
    def _last():
        sl = NT // 2 - 1
        row0 = (NT - 1) * T
        g = _upk(g_s[...])
        w2_part(0, sl, 0, NSPLIT, g=g)
        ys = []
        attention(1, row0, CHAINL, 0, T, hooks={TH: lambda tok: ys.append(wo_mm(1, sl, 0, TH)),
                                                 HKL: lambda tok: ys.append(ln2_after(1, 0, TH, tok))})
        ya = ys[1]
        w2_part(0, sl, NSPLIT, D, g=g)
        w1_gelu(ya, 0, TH)
        yb = wo_ln2(1, sl, TH, TH)
        w2_part(1, sl, 0, D, 0, TH)
        w1_gelu(yb, TH, TH)
        x_out_copy(0, sl).start()
        x_out_copy(1, sl, 0, TH).start()
        w2_part(1, sl, 0, D, TH, TH)
        x_out_copy(1, sl, TH, TH, 1).start()
        for t in range(NT - 1):
            x_out_copy(t % 2, t // 2).wait()
        x_out_copy(1, sl, 0, TH).wait()
        x_out_copy(1, sl, TH, TH, 1).wait()


@jax.jit
def pallas_interleave_layers__sliding_local_dilated__mixer_channel_mlp__prompt_kernel(
    A_x, A_wqkv, A_wo, B_x, B_w1, B_b1, B_w2, B_b2,
):
    del B_x
    any_spec = pl.BlockSpec(memory_space=pl.ANY)
    kv = pltpu.VMEM((NL, HALO + T, 128), F32)
    td = pltpu.VMEM((T, D), F32)
    tq = pltpu.VMEM((T + 8, D), F32)
    return pl.pallas_call(
        _kernel,
        grid=(int(os.environ.get('G', NSTEPS)),),
        in_specs=[any_spec] * 7,
        out_specs=any_spec,
        out_shape=jax.ShapeDtypeStruct((1, S, D), A_x.dtype),
        scratch_shapes=[
            pltpu.VMEM((S // 2, D), BF16),
            pltpu.VMEM((S // 2, D), BF16),
            pltpu.VMEM((3, D, D), BF16),
            pltpu.VMEM((D, D), BF16),
            pltpu.VMEM((NL, F, 128), BF16),
            pltpu.VMEM((NL, F, 128), BF16),
            pltpu.VMEM((F,), BF16),
            pltpu.VMEM((D,), BF16),
            pltpu.VMEM((3 * D // 2, D), U32),
            pltpu.VMEM((D // 2, D), U32),
            tq, kv, kv, tq, kv, kv,
            tq, tq,
            pltpu.VMEM((T // 2, F), U32),
            pltpu.VMEM((T // 2, D), U32),
            pltpu.VMEM((T // 2, D), U32),
            td,
            pltpu.SemaphoreType.DMA((NSEM,)),
        ],
        compiler_params=pltpu.CompilerParams(
            dimension_semantics=("arbitrary",),
            vmem_limit_bytes=100 * 1024 * 1024,
        ),
    )(A_x, A_wqkv, A_wo, B_w1.T, B_b1, B_w2, B_b2)
```

```python
import math

import jax
import jax.numpy as jnp
from jax import lax
import jax.experimental.pallas as pl
import jax.experimental.pallas.tpu as pltpu

S, D, F = 2048, 512, 1376
H, DH, W, DIL = 32, 16, 8, 2
EPS = 1e-5

T = 256
TH = T // 2
R = 8
HALO = 16
NL = D // 128
NT = S // T
NITEMS = 2 * NT
NSTEPS = NITEMS // 2 + 1

NSPLIT = 384
CHAIN = 3
QS, KS, V0, RA = 256, 896, 1408, 208
HKL = 168
LS = 384

F32 = jnp.float32
BF16 = jnp.bfloat16
U32 = jnp.uint32
NT_DIMS = (((1,), (1,)), ((), ()))
LOG2E = math.log2(math.e)

SEM_X0, SEM_WQ0, SEM_WQ1, SEM_WK, SEM_WV, SEM_W1, SEM_W2, SEM_X2, SEM_OUT = range(9)
NSEM = 9


def _pk(x):
    return pltpu.bitcast(x, U32)


def _upk(x):
    return pltpu.bitcast(x, BF16)


def _ln(x):
    m = jnp.mean(x, axis=-1, keepdims=True)
    xc = x - m
    v = jnp.mean(xc * xc, axis=-1, keepdims=True)
    return xc * lax.rsqrt(v + EPS)


def _ln_ln(x):
    m = jnp.mean(x, axis=-1, keepdims=True)
    xc = x - m
    v = jnp.mean(xc * xc, axis=-1, keepdims=True)
    return xc * lax.rsqrt(v * (1.0 + EPS) + EPS * EPS)


def _gelu(x):
    c0 = math.sqrt(2.0 / math.pi)
    c1 = c0 * 0.044715
    u = x * (c0 + c1 * (x * x))
    hx = 0.5 * x
    return hx + hx * jnp.tanh(u)


def _fold(op, xs):
    acc = xs[0]
    for x in xs[1:]:
        acc = op(acc, x)
    return acc


def _kernel(x_hbm, wqkv_hbm, wo_hbm, w1t_hbm, b1_hbm, w2_hbm, b2_hbm, out_hbm,
            xe, xo, wqkv_raw, wo_raw, w1t_s, w2_s, b1_s, b2_s, wqkv_p, wo_p,
            qa, ka, va, qb, kb, vb, x1a, x1b, g_s, xn0_s, xn1_s, o_s, sems):
    step = pl.program_id(0)
    xbuf = (xe, xo)
    qs, ks, vs, x1s = (qa, qb), (ka, kb), (va, vb), (x1a, x1b)

    def rows_at(slot, r0, n):
        if isinstance(slot, int):
            return pl.ds(slot * T + r0, n)
        return pl.ds(pl.multiple_of(slot * T + r0, TH), n)

    def x_in_copy(t):
        sem = (SEM_X0, SEM_WV, SEM_W2, SEM_W2, SEM_X2, SEM_X2, SEM_X2, SEM_X2)[t]
        return pltpu.make_async_copy(
            x_hbm.at[0, pl.ds(t * T, T), :], xbuf[t % 2].at[pl.ds((t // 2) * T, T), :], sems.at[sem])

    def x_out_copy(par, slot, r0=0, n=T, c0=0, c1=D):
        return pltpu.make_async_copy(
            xbuf[par].at[rows_at(slot, r0, n), pl.ds(c0, c1 - c0)],
            out_hbm.at[0, rows_at(2 * slot + par, r0, n), pl.ds(c0, c1 - c0)],
            sems.at[SEM_OUT])

    def wqkv_copy(b, sem, r0=0, n=D):
        return pltpu.make_async_copy(
            wqkv_hbm.at[pl.ds(r0, n), pl.ds(b * D, D)], wqkv_raw.at[b, pl.ds(r0, n), :], sems.at[sem])

    def col_copies(src, dst, sem):
        return [pltpu.make_async_copy(src.at[:, pl.ds(j * 128, 128)], dst.at[j], sems.at[sem])
                for j in range(NL)]

    def w1_group():
        return (col_copies(wo_hbm, wo_raw, SEM_W1) + col_copies(w1t_hbm, w1t_s, SEM_W1)
                + [pltpu.make_async_copy(b1_hbm, b1_s, sems.at[SEM_W1])])

    def w2_group():
        return (col_copies(w2_hbm, w2_s, SEM_W2)
                + [pltpu.make_async_copy(b2_hbm, b2_s, sems.at[SEM_W2]), x_in_copy(2), x_in_copy(3)])

    def wcols(ref, j0, j1):
        return jnp.concatenate([_upk(ref.at[j].bitcast(U32)[...]) for j in range(j0, j1)], axis=1)

    def load_x(par, slot, r0=0, n=T):
        return xbuf[par][rows_at(slot, r0, n), :].astype(F32)

    def zoff(k):
        return pl.multiple_of(lax.shift_right_logical(step, k) * 8, 8)

    def proj(xn, par, c0, c1, r0=0, n=T):
        qscale = (DH ** -0.5) * LOG2E
        res = jnp.dot(xn, _upk(wqkv_p[:, c0:c1]), preferred_element_type=F32)
        for c in range(c0, c1, 128):
            blk = res[:, c - c0:c - c0 + 128]
            b, j = c // D, (c % D) // 128
            if b == 0:
                qs[par][r0:r0 + n, j * 128:(j + 1) * 128] = blk * qscale
            elif b == 1:
                ks[par][j, HALO + r0:HALO + r0 + n, :] = blk
            else:
                vs[par][j, HALO + r0:HALO + r0 + n, :] = blk

    def halo_copy(par):
        for j in range(NL):
            ks[par][j, 0:HALO, :] = ks[1 - par][j, T:T + HALO, :]
            vs[par][j, 0:HALO, :] = vs[1 - par][j, T:T + HALO, :]

    def attention(par, row0, chain, ra=0, rb=T, hooks=None):
        q_s, k_s, v_s = qs[par], ks[par], vs[par]
        chunks = list(range(ra // R, rb // R))
        z1, z2 = zoff(10), zoff(11)

        def load_q(c):
            qq = q_s[pl.ds(z1 + c * R, R), :]
            return [qq[:, j * 128:(j + 1) * 128] for j in range(NL)]

        pend = {c: load_q(c) for c in chunks[:chain]}
        for c in chunks:
            r0 = c * R
            q = pend.pop(c)
            logits = []
            for w in range(W):
                st = HALO + r0 - DIL * w
                acc = _fold(jnp.add, [q[j] * k_s[j, st:st + R, :] for j in range(NL)])
                acc = acc + pltpu.roll(acc, 64, 1)
                acc = acc + pltpu.roll(acc, 32, 1)
                if r0 < DIL * w:
                    row = lax.broadcasted_iota(jnp.int32, (R, 128), 0) + (row0 + r0)
                    acc = jnp.where(row >= DIL * w, acc, -1e9 * LOG2E)
                logits.append(acc)
            m = _fold(jnp.maximum, logits)
            ps = [jnp.exp2(lg - m) for lg in logits]
            inv = pl.reciprocal(_fold(jnp.add, ps), approx=True)
            outs = []
            for j in range(NL):
                acc = _fold(jnp.add, [ps[w] * v_s[j, HALO + r0 - DIL * w:HALO + r0 - DIL * w + R, :]
                                      for w in range(W)])
                outs.append(acc * inv)
            o_s[r0:r0 + R, :] = jnp.concatenate(outs, axis=1)
            q_s[pl.ds(z2 + T, 8), 0:128] = outs[NL - 1]
            if c + chain <= chunks[-1]:
                pend[c + chain] = load_q(c + chain)
            if hooks and (r0 + R) in hooks:
                hooks[r0 + R](outs[NL - 1])

    def w2_part(par, slot, c0, c1, r0=0, n=T, g=None):
        if g is None:
            g = _upk(g_s[r0 // 2:(r0 + n) // 2, :])
        b2 = b2_s[...].astype(F32)[None, :]
        acc = jnp.dot(g, wcols(w2_s, c0 // 128, c1 // 128), preferred_element_type=F32)
        x2 = x1s[par][r0:r0 + n, c0:c1] + (acc + b2[:, c0:c1])
        xbuf[par][rows_at(slot, r0, n), c0:c1] = x2.astype(BF16)

    def wo_mm(par, slot, r0=0, n=T):
        o = o_s[r0:r0 + n, :].astype(BF16)
        x1 = load_x(par, slot, r0, n) + jnp.dot(o, _upk(wo_p[...]), preferred_element_type=F32)
        x1s[par][r0:r0 + n, :] = x1
        return x1

    def ln2_after(par, r0, n, tok):
        x1s[par][pl.ds(zoff(11) + T, 8), 0:128] = tok
        return _ln_ln(x1s[par][pl.ds(zoff(10) + r0, n), :]).astype(BF16)

    def wo_ln2(par, slot, r0=0, n=T):
        return _ln_ln(wo_mm(par, slot, r0, n)).astype(BF16)

    def w1_gelu(y, r0=0, n=T):
        b1 = b1_s[...].astype(F32)[None, :]
        h = lax.dot_general(y, wcols(w1t_s, 0, NL), NT_DIMS, preferred_element_type=F32) + b1
        gl = _gelu(h)
        g_s[r0 // 2:(r0 + n) // 2, :] = _pk(gl.astype(BF16))
        return gl

    def slot_body(sig, par, pace_next):
        slot_b = (sig % NT) // 2
        slot_c = ((sig + NT - 1) % NT) // 2
        slot_a = ((sig + 1) % NT) // 2
        xa = load_x(1 - par, slot_a)
        g = _upk(g_s[...])
        w2_part(1 - par, slot_c, 0, NSPLIT, g=g)
        proj(_ln(xa).astype(BF16), 1 - par, 0, 3 * D)
        halo_copy(1 - par)
        attention(par, (sig % NT) * T, CHAIN)
        y = wo_ln2(par, slot_b)
        w2_part(1 - par, slot_c, NSPLIT, D, g=g)
        gl = w1_gelu(y)
        if pace_next:
            tok = gl[T - 16:T, F - 96:F]
            qs[1 - par][pl.ds(zoff(11) + T, 8), 0:96] = tok[8:16]
            xbuf[par][pl.ds(pl.multiple_of(zoff(11) * 2 + S // 2, 16), 16), 0:96] = tok.astype(BF16)

    def prep_qkv(b, r0=0, n=D):
        w = _pk(wqkv_raw[b, r0:r0 + n, :])
        lane = lax.broadcasted_iota(jnp.int32, (n // 2, 128), 1)
        a_src = (lane // 4) % 4
        for j in range(NL):
            acc = w[:, 0:128]
            for J in range(1, NL):
                acc = jnp.where(a_src == (j + J) % 4, w[:, J * 128:(J + 1) * 128], acc)
            idx = (lane % 8) * 16 + 4 * ((lane // 8 + j) % 4) + lane // 32
            wqkv_p[r0 // 2:(r0 + n) // 2, b * D + j * 128:b * D + (j + 1) * 128] = (
                jnp.take_along_axis(acc, idx, axis=1))

    def prep_wo():
        lo = jnp.uint32(0xFFFF)
        hi = jnp.uint32(0xFFFF0000)
        grp = lax.broadcasted_iota(jnp.int32, (16, 128), 0) // 4
        for c in range(NL):
            src32 = wo_raw.at[c].bitcast(U32)
            blk = []
            for t in range(DH // 2):
                ev = src32[pl.ds(t, 16, stride=16), :]
                od = src32[pl.ds(8 + t, 16, stride=16), :]
                blk.append((ev & lo) | (od << 16))
                blk.append((ev >> 16) | (od & hi))
            for j in range(NL):
                for e in range(4):
                    acc = blk[4 * j + e]
                    for J in range(1, NL):
                        acc = jnp.where(grp == J, blk[4 * ((j + J) % 4) + e], acc)
                    wo_p[j * 64 + e * 16:j * 64 + (e + 1) * 16, c * 128:(c + 1) * 128] = acc

    @pl.when(step == 0)
    def _first():
        wq0 = wqkv_copy(0, SEM_WQ0, 0, D // 2)
        wq1 = wqkv_copy(0, SEM_WQ1, D // 2, D // 2)
        wk = wqkv_copy(1, SEM_WK)
        wv = wqkv_copy(2, SEM_WV)
        for c in ([x_in_copy(0), wq0, wq1, wk, wv, x_in_copy(1)] + w1_group() + w2_group()
                  + [x_in_copy(t) for t in range(4, NT)]):
            c.start()
        z = jnp.zeros((HALO, 128), F32)
        for j in range(NL):
            ka[j, 0:HALO, :] = z
            va[j, 0:HALO, :] = z
        x_in_copy(0).wait()
        xn0_s[...] = _pk(_ln(load_x(0, 0)).astype(BF16))
        wq0.wait()
        prep_qkv(0, 0, D // 2)
        wq1.wait()
        prep_qkv(0, D // 2, D // 2)
        proj(_upk(xn0_s[...]), 0, 0, QS)
        wk.wait()
        prep_qkv(1)
        proj(_upk(xn0_s[...]), 0, QS, KS)
        wv.wait()
        x_in_copy(1).wait()
        prep_qkv(2)
        proj(_upk(xn0_s[...]), 0, KS, 2 * D)
        proj(_upk(xn0_s[0:TH // 2, :]), 0, 2 * D, 3 * D, 0, TH)
        proj(_upk(xn0_s[TH // 2:T // 2, :]), 0, 2 * D, 3 * D, TH, TH)
        xn1 = _ln(load_x(1, 0)).astype(BF16)
        xn1_s[...] = _pk(xn1)
        proj(xn1, 1, 0, V0)
        attention(0, 0, CHAIN, 0, RA)
        for c in w1_group():
            c.wait()
        prep_wo()
        proj(_upk(xn1_s[...]), 1, V0, 3 * D)
        halo_copy(1)
        wo_mm(0, 0, 0, TH)
        ys = []
        attention(0, 0, 2 * CHAIN, RA, T, hooks={T: lambda tok: ys.append(ln2_after(0, 0, TH, tok))})
        yb = wo_ln2(0, 0, TH, TH)
        w1_gelu(ys[0], 0, TH)
        w1_gelu(yb, TH, TH)
        for c in w2_group():
            c.wait()

    @pl.when(step == 2)
    def _():
        for t in range(4, NT):
            x_in_copy(t).wait()

    @pl.when(jnp.logical_and(step > 0, step < NSTEPS - 1))
    def _mid():
        slot_body(2 * step - 1, 1, True)
        slot_body(2 * step, 0, False)

    for _slot in range(NT // 2 - 1):
        @pl.when(step == NT // 2 + 1 + _slot)
        def _(slot=_slot):
            x_out_copy(0, slot).start()
            x_out_copy(1, slot).start()

    @pl.when(step == NSTEPS - 1)
    def _last():
        sl = NT // 2 - 1
        g = _upk(g_s[...])
        w2_part(0, sl, 0, NSPLIT, g=g)
        ys = []
        attention(1, (NT - 1) * T, CHAIN, 0, T,
                  hooks={TH: lambda tok: wo_mm(1, sl, 0, TH),
                         HKL: lambda tok: ys.append(ln2_after(1, 0, TH, tok))})
        w2_part(0, sl, NSPLIT, D, g=g)
        w1_gelu(ys[0], 0, TH)
        yb = wo_ln2(1, sl, TH, TH)
        w2_part(1, sl, 0, D, 0, TH)
        w1_gelu(yb, TH, TH)
        tail = [x_out_copy(0, sl), x_out_copy(1, sl, 0, TH),
                x_out_copy(1, sl, TH, TH, 0, LS), x_out_copy(1, sl, TH, TH, LS, D)]
        tail[0].start()
        tail[1].start()
        w2_part(1, sl, 0, LS, TH, TH)
        tail[2].start()
        w2_part(1, sl, LS, D, TH, TH)
        tail[3].start()
        for t in range(NT - 2):
            x_out_copy(t % 2, t // 2).wait()
        for c in tail:
            c.wait()


@jax.jit
def pallas_interleave_layers__sliding_local_dilated__mixer_channel_mlp__prompt_kernel(
    A_x: jax.Array,
    A_wqkv: jax.Array,
    A_wo: jax.Array,
    B_x: jax.Array,
    B_w1: jax.Array,
    B_b1: jax.Array,
    B_w2: jax.Array,
    B_b2: jax.Array,
):
    del B_x
    any_spec = pl.BlockSpec(memory_space=pl.ANY)
    kv = pltpu.VMEM((NL, HALO + T, 128), F32)
    tq = pltpu.VMEM((T + 8, D), F32)
    return pl.pallas_call(
        _kernel,
        grid=(NSTEPS,),
        in_specs=[any_spec] * 7,
        out_specs=any_spec,
        out_shape=jax.ShapeDtypeStruct((1, S, D), A_x.dtype),
        scratch_shapes=[
            pltpu.VMEM((S // 2 + 16, D), BF16),
            pltpu.VMEM((S // 2 + 16, D), BF16),
            pltpu.VMEM((3, D, D), BF16),
            pltpu.VMEM((NL, D, 128), BF16),
            pltpu.VMEM((NL, F, 128), BF16),
            pltpu.VMEM((NL, F, 128), BF16),
            pltpu.VMEM((F,), BF16),
            pltpu.VMEM((D,), BF16),
            pltpu.VMEM((D // 2, 3 * D), U32),
            pltpu.VMEM((D // 2, D), U32),
            tq, kv, kv, tq, kv, kv,
            tq, tq,
            pltpu.VMEM((T // 2, F), U32),
            pltpu.VMEM((T // 2, D), U32),
            pltpu.VMEM((T // 2, D), U32),
            pltpu.VMEM((T, D), F32),
            pltpu.SemaphoreType.DMA((NSEM,)),
        ],
        compiler_params=pltpu.CompilerParams(
            dimension_semantics=("arbitrary",),
            vmem_limit_bytes=64 * 1024 * 1024,
        ),
    )(A_x, A_wqkv, A_wo, B_w1.T, B_b1, B_w2, B_b2)
```

```python
import math

import jax
import jax.numpy as jnp
from jax import lax
import jax.experimental.pallas as pl
import jax.experimental.pallas.tpu as pltpu

S, D, F = 2048, 512, 1376
H, DH, W, DIL = 32, 16, 8, 2
EPS = 1e-5

T = 256
TH = T // 2
R = 8
HALO = 16
NL = D // 128
NT = S // T
NITEMS = 2 * NT
NSTEPS = NITEMS // 2 + 1

NSPLIT = 384
CHAIN = 3
QS, KS, V0, RA = 256, 896, 1408, 208
HKL = 168
LS = 256

F32 = jnp.float32
BF16 = jnp.bfloat16
U32 = jnp.uint32
NT_DIMS = (((1,), (1,)), ((), ()))
LOG2E = math.log2(math.e)

SEM_X0, SEM_WQ0, SEM_WQ1, SEM_WK, SEM_WV, SEM_W1, SEM_W2, SEM_X2 = range(8)
SEM_OUT = SEM_X0
NSEM = 8


def _pk(x):
    return pltpu.bitcast(x, U32)


def _upk(x):
    return pltpu.bitcast(x, BF16)


def _ln(x):
    m = jnp.mean(x, axis=-1, keepdims=True)
    xc = x - m
    v = jnp.mean(xc * xc, axis=-1, keepdims=True)
    return xc * lax.rsqrt(v + EPS)


def _ln_ln(x):
    m = jnp.mean(x, axis=-1, keepdims=True)
    xc = x - m
    v = jnp.mean(xc * xc, axis=-1, keepdims=True)
    return xc * lax.rsqrt(v * (1.0 + EPS) + EPS * EPS)


def _gelu(x):
    c0 = math.sqrt(2.0 / math.pi)
    c1 = c0 * 0.044715
    u = x * (c0 + c1 * (x * x))
    hx = 0.5 * x
    return hx + hx * jnp.tanh(u)


def _fold(op, xs):
    acc = xs[0]
    for x in xs[1:]:
        acc = op(acc, x)
    return acc


def _kernel(x_hbm, wqkv_hbm, wo_hbm, w1t_hbm, b1_hbm, w2_hbm, b2_hbm, out_hbm,
            xe, xo, wqkv_raw, wo_raw, w1t_s, b1_s, b2_s, wqkv_p, wo_p,
            qa, ka, va, qb, kb, vb, x1a, x1b, g_s, xn0_s, xn1_s, o_s, wo32, w1t_raw, w2_s, sems):
    step = pl.program_id(0)
    xbuf = (xe, xo)
    qs, ks, vs, x1s = (qa, qb), (ka, kb), (va, vb), (x1a, x1b)

    def rows_at(slot, r0, n):
        if isinstance(slot, int):
            return pl.ds(slot * T + r0, n)
        return pl.ds(pl.multiple_of(slot * T + r0, TH), n)

    def x_in_copy(t):
        sem = (SEM_X0, SEM_WV, SEM_W2, SEM_W2, SEM_X2, SEM_X2, SEM_X2, SEM_X2)[t]
        return pltpu.make_async_copy(
            x_hbm.at[0, pl.ds(t * T, T), :], xbuf[t % 2].at[pl.ds((t // 2) * T, T), :], sems.at[sem])

    def x_out_copy(par, slot, r0=0, n=T, c0=0, c1=D):
        return pltpu.make_async_copy(
            xbuf[par].at[rows_at(slot, r0, n), pl.ds(c0, c1 - c0)],
            out_hbm.at[0, rows_at(2 * slot + par, r0, n), pl.ds(c0, c1 - c0)],
            sems.at[SEM_OUT])

    def wqkv_copy(b, sem, r0=0, n=D):
        return pltpu.make_async_copy(
            wqkv_hbm.at[pl.ds(r0, n), pl.ds(b * D, D)], wqkv_raw.at[b, pl.ds(r0, n), :], sems.at[sem])

    def w1_group():
        return [pltpu.make_async_copy(wo_hbm, wo_raw, sems.at[SEM_W1]),
                pltpu.make_async_copy(w1t_hbm, w1t_raw, sems.at[SEM_W1]),
                pltpu.make_async_copy(b1_hbm, b1_s, sems.at[SEM_W1])]

    def w2_group():
        return [pltpu.make_async_copy(w2_hbm, w2_s, sems.at[SEM_W2]),
                pltpu.make_async_copy(b2_hbm, b2_s, sems.at[SEM_W2]),
                x_in_copy(2), x_in_copy(3)]

    def load_x(par, slot, r0=0, n=T):
        return xbuf[par][rows_at(slot, r0, n), :].astype(F32)

    def zoff(k):
        return pl.multiple_of(lax.shift_right_logical(step, k) * 8, 8)

    def proj(xn, par, c0, c1, r0=0, n=T):
        qscale = (DH ** -0.5) * LOG2E
        res = jnp.dot(xn, _upk(wqkv_p[:, c0:c1]), preferred_element_type=F32)
        for c in range(c0, c1, 128):
            blk = res[:, c - c0:c - c0 + 128]
            b, j = c // D, (c % D) // 128
            if b == 0:
                qs[par][r0:r0 + n, j * 128:(j + 1) * 128] = blk * qscale
            elif b == 1:
                ks[par][j, HALO + r0:HALO + r0 + n, :] = blk
            else:
                vs[par][j, HALO + r0:HALO + r0 + n, :] = blk

    def halo_copy(par):
        for j in range(NL):
            ks[par][j, 0:HALO, :] = ks[1 - par][j, T:T + HALO, :]
            vs[par][j, 0:HALO, :] = vs[1 - par][j, T:T + HALO, :]

    def attention(par, row0, chain, ra=0, rb=T, hooks=None):
        q_s, k_s, v_s = qs[par], ks[par], vs[par]
        chunks = list(range(ra // R, rb // R))
        z1, z2 = zoff(10), zoff(11)

        def load_q(c):
            qq = q_s[pl.ds(z1 + c * R, R), :]
            return [qq[:, j * 128:(j + 1) * 128] for j in range(NL)]

        pend = {c: load_q(c) for c in chunks[:chain]}
        for c in chunks:
            r0 = c * R
            q = pend.pop(c)
            logits = []
            for w in range(W):
                st = HALO + r0 - DIL * w
                acc = _fold(jnp.add, [q[j] * k_s[j, st:st + R, :] for j in range(NL)])
                acc = acc + pltpu.roll(acc, 64, 1)
                acc = acc + pltpu.roll(acc, 32, 1)
                if r0 < DIL * w:
                    row = lax.broadcasted_iota(jnp.int32, (R, 128), 0) + (row0 + r0)
                    acc = jnp.where(row >= DIL * w, acc, -1e9 * LOG2E)
                logits.append(acc)
            m = _fold(jnp.maximum, logits)
            ps = [jnp.exp2(lg - m) for lg in logits]
            inv = pl.reciprocal(_fold(jnp.add, ps), approx=True)
            outs = []
            for j in range(NL):
                acc = _fold(jnp.add, [ps[w] * v_s[j, HALO + r0 - DIL * w:HALO + r0 - DIL * w + R, :]
                                      for w in range(W)])
                outs.append(acc * inv)
            o_s[r0:r0 + R, :] = jnp.concatenate(outs, axis=1)
            q_s[pl.ds(z2 + T, 8), 0:128] = outs[1]
            if c + chain <= chunks[-1]:
                pend[c + chain] = load_q(c + chain)
            if hooks and (r0 + R) in hooks:
                hooks[r0 + R](outs[NL - 1])

    def w2_part(par, slot, c0, c1, r0=0, n=T, g=None):
        if g is None:
            g = _upk(g_s[r0 // 2:(r0 + n) // 2, :])
        b2 = b2_s[...].astype(F32)[None, :]
        acc = jnp.dot(g, w2_s[:, c0:c1], preferred_element_type=F32)
        x2 = x1s[par][r0:r0 + n, c0:c1] + (acc + b2[:, c0:c1])
        xbuf[par][rows_at(slot, r0, n), c0:c1] = x2.astype(BF16)

    def wo_mm(par, slot, r0=0, n=T):
        o = o_s[r0:r0 + n, :].astype(BF16)
        x1 = load_x(par, slot, r0, n) + jnp.dot(o, _upk(wo_p[...]), preferred_element_type=F32)
        x1s[par][r0:r0 + n, :] = x1
        return x1

    def ln2_after(par, r0, n, tok):
        x1s[par][pl.ds(zoff(11) + T, 8), 0:128] = tok
        return _ln_ln(x1s[par][pl.ds(zoff(10) + r0, n), :]).astype(BF16)

    def wo_ln2(par, slot, r0=0, n=T):
        return _ln_ln(wo_mm(par, slot, r0, n)).astype(BF16)

    def w1_gelu(y, r0=0, n=T):
        b1 = b1_s[...].astype(F32)[None, :]
        h = lax.dot_general(y, _upk(w1t_s[...]), NT_DIMS, preferred_element_type=F32) + b1
        gl = _gelu(h)
        g_s[r0 // 2:(r0 + n) // 2, :] = _pk(gl.astype(BF16))
        return gl

    def slot_body(sig, par, pace_next):
        slot_b = (sig % NT) // 2
        slot_c = ((sig + NT - 1) % NT) // 2
        slot_a = ((sig + 1) % NT) // 2
        xa = load_x(1 - par, slot_a)
        g = _upk(g_s[...])
        w2_part(1 - par, slot_c, 0, NSPLIT, g=g)
        proj(_ln(xa).astype(BF16), 1 - par, 0, 3 * D)
        halo_copy(1 - par)
        attention(par, (sig % NT) * T, CHAIN)
        y = wo_ln2(par, slot_b)
        w2_part(1 - par, slot_c, NSPLIT, D, g=g)
        gl = w1_gelu(y)
        if pace_next:
            tok = gl[T - 16:T, F - 96:F]
            qs[1 - par][pl.ds(zoff(11) + T, 8), 0:96] = tok[8:16]
            xbuf[par][pl.ds(pl.multiple_of(zoff(11) * 2 + S // 2, 16), 16), 0:96] = tok.astype(BF16)

    def prep_qkv(b, r0=0, n=D):
        w = _pk(wqkv_raw[b, r0:r0 + n, :])
        lane = lax.broadcasted_iota(jnp.int32, (n // 2, 128), 1)
        a_src = (lane // 4) % 4
        for j in range(NL):
            acc = w[:, 0:128]
            for J in range(1, NL):
                acc = jnp.where(a_src == (j + J) % 4, w[:, J * 128:(J + 1) * 128], acc)
            idx = (lane % 8) * 16 + 4 * ((lane // 8 + j) % 4) + lane // 32
            wqkv_p[r0 // 2:(r0 + n) // 2, b * D + j * 128:b * D + (j + 1) * 128] = (
                jnp.take_along_axis(acc, idx, axis=1))

    def prep_wo():
        lo = jnp.uint32(0xFFFF)
        hi = jnp.uint32(0xFFFF0000)
        grp = lax.broadcasted_iota(jnp.int32, (16, 128), 0) // 4
        for c in range(NL):
            wo32[c] = _pk(wo_raw[:, c * 128:(c + 1) * 128])
            src32 = wo32.at[c]
            blk = []
            for t in range(DH // 2):
                ev = src32[pl.ds(t, 16, stride=16), :]
                od = src32[pl.ds(8 + t, 16, stride=16), :]
                blk.append((ev & lo) | (od << 16))
                blk.append((ev >> 16) | (od & hi))
            for j in range(NL):
                for e in range(4):
                    acc = blk[4 * j + e]
                    for J in range(1, NL):
                        acc = jnp.where(grp == J, blk[4 * ((j + J) % 4) + e], acc)
                    wo_p[j * 64 + e * 16:j * 64 + (e + 1) * 16, c * 128:(c + 1) * 128] = acc

    @pl.when(step == 0)
    def _first():
        wq0 = wqkv_copy(0, SEM_WQ0, 0, D // 2)
        wq1 = wqkv_copy(0, SEM_WQ1, D // 2, D // 2)
        wk = wqkv_copy(1, SEM_WK)
        wv = wqkv_copy(2, SEM_WV)
        for c in ([x_in_copy(0), wq0, wq1, wk, wv, x_in_copy(1)] + w1_group() + w2_group()
                  + [x_in_copy(t) for t in range(4, NT)]):
            c.start()
        z = jnp.zeros((HALO, 128), F32)
        for j in range(NL):
            ka[j, 0:HALO, :] = z
            va[j, 0:HALO, :] = z
        x_in_copy(0).wait()
        xn0_s[...] = _pk(_ln(load_x(0, 0)).astype(BF16))
        wq0.wait()
        prep_qkv(0, 0, D // 2)
        wq1.wait()
        prep_qkv(0, D // 2, D // 2)
        proj(_upk(xn0_s[...]), 0, 0, QS)
        wk.wait()
        prep_qkv(1)
        proj(_upk(xn0_s[...]), 0, QS, KS)
        wv.wait()
        x_in_copy(1).wait()
        prep_qkv(2)
        proj(_upk(xn0_s[...]), 0, KS, 2 * D)
        proj(_upk(xn0_s[0:TH // 2, :]), 0, 2 * D, 3 * D, 0, TH)
        proj(_upk(xn0_s[TH // 2:T // 2, :]), 0, 2 * D, 3 * D, TH, TH)
        xn1 = _ln(load_x(1, 0)).astype(BF16)
        xn1_s[...] = _pk(xn1)
        proj(xn1, 1, 0, V0)
        attention(0, 0, CHAIN, 0, RA)
        for c in w1_group():
            c.wait()
        prep_wo()
        w1t_s[...] = _pk(w1t_raw[...])
        proj(_upk(xn1_s[...]), 1, V0, 3 * D)
        halo_copy(1)
        wo_mm(0, 0, 0, TH)
        ys = []
        attention(0, 0, 2 * CHAIN, RA, T, hooks={T: lambda tok: ys.append(ln2_after(0, 0, TH, tok))})
        yb = wo_ln2(0, 0, TH, TH)
        w1_gelu(ys[0], 0, TH)
        w1_gelu(yb, TH, TH)
        for c in w2_group():
            c.wait()

    @pl.when(step == 2)
    def _():
        for t in range(4, NT):
            x_in_copy(t).wait()

    @pl.when(jnp.logical_and(step > 0, step < NSTEPS - 1))
    def _mid():
        slot_body(2 * step - 1, 1, True)
        slot_body(2 * step, 0, False)

    for _slot in range(NT // 2 - 1):
        @pl.when(step == NT // 2 + 1 + _slot)
        def _(slot=_slot):
            x_out_copy(0, slot).start()
            x_out_copy(1, slot).start()

    @pl.when(step == NSTEPS - 1)
    def _last():
        sl = NT // 2 - 1
        g = _upk(g_s[...])
        w2_part(0, sl, 0, NSPLIT, g=g)
        ys = []
        attention(1, (NT - 1) * T, CHAIN, 0, T,
                  hooks={TH: lambda tok: wo_mm(1, sl, 0, TH),
                         HKL: lambda tok: ys.append(ln2_after(1, 0, TH, tok))})
        w2_part(0, sl, NSPLIT, D, g=g)
        w1_gelu(ys[0], 0, TH)
        yb = wo_ln2(1, sl, TH, TH)
        w2_part(1, sl, 0, D, 0, TH)
        w1_gelu(yb, TH, TH)
        tail = [x_out_copy(0, sl), x_out_copy(1, sl, 0, TH),
                x_out_copy(1, sl, TH, TH, 0, LS), x_out_copy(1, sl, TH, TH, LS, D)]
        tail[0].start()
        tail[1].start()
        w2_part(1, sl, 0, LS, TH, TH)
        tail[2].start()
        w2_part(1, sl, LS, D, TH, TH)
        tail[3].start()
        for t in range(NT - 2):
            x_out_copy(t % 2, t // 2).wait()
        for c in tail:
            c.wait()


@jax.jit
def pallas_interleave_layers__sliding_local_dilated__mixer_channel_mlp__prompt_kernel(
    A_x: jax.Array,
    A_wqkv: jax.Array,
    A_wo: jax.Array,
    B_x: jax.Array,
    B_w1: jax.Array,
    B_b1: jax.Array,
    B_w2: jax.Array,
    B_b2: jax.Array,
):
    del B_x
    any_spec = pl.BlockSpec(memory_space=pl.ANY)
    kv = pltpu.VMEM((NL, HALO + T, 128), F32)
    tq = pltpu.VMEM((T + 8, D), F32)
    return pl.pallas_call(
        _kernel,
        grid=(NSTEPS,),
        in_specs=[any_spec] * 7,
        out_specs=any_spec,
        out_shape=jax.ShapeDtypeStruct((1, S, D), A_x.dtype),
        scratch_shapes=[
            pltpu.VMEM((S // 2 + 16, D), BF16),
            pltpu.VMEM((S // 2 + 16, D), BF16),
            pltpu.VMEM((3, D, D), BF16),
            pltpu.VMEM((D, D), BF16),
            pltpu.VMEM((F // 2, D), U32),
            pltpu.VMEM((F,), BF16),
            pltpu.VMEM((D,), BF16),
            pltpu.VMEM((D // 2, 3 * D), U32),
            pltpu.VMEM((D // 2, D), U32),
            tq, kv, kv, tq, kv, kv,
            tq, tq,
            pltpu.VMEM((T // 2, F), U32),
            pltpu.VMEM((T // 2, D), U32),
            pltpu.VMEM((T // 2, D), U32),
            pltpu.VMEM((T, D), F32),
            pltpu.VMEM((NL, D // 2, 128), U32),
            pltpu.VMEM((F, D), BF16),
            pltpu.VMEM((F, D), BF16),
            pltpu.SemaphoreType.DMA((NSEM,)),
        ],
        compiler_params=pltpu.CompilerParams(
            dimension_semantics=("arbitrary",),
            vmem_limit_bytes=64 * 1024 * 1024,
        ),
    )(A_x, A_wqkv, A_wo, B_w1.T, B_b1, B_w2, B_b2)
```

```python
import math

import jax
import jax.numpy as jnp
from jax import lax
import jax.experimental.pallas as pl
import jax.experimental.pallas.tpu as pltpu

S, D, F = 2048, 512, 1376
H, DH, W, DIL = 32, 16, 8, 2
EPS = 1e-5

T = 256
TH = T // 2
R = 8
HALO = 16
NL = D // 128
NT = S // T
NITEMS = 2 * NT
NSTEPS = NITEMS // 2 + 1

NSPLIT = 384
CHAIN = 3
QS, KS, V0, RA = 256, 896, 1408, 208
HKL = 168
LS = 256

F32 = jnp.float32
BF16 = jnp.bfloat16
U32 = jnp.uint32
NT_DIMS = (((1,), (1,)), ((), ()))
LOG2E = math.log2(math.e)

SEM_X0, SEM_WQ0, SEM_WQ1, SEM_WK, SEM_WV, SEM_W1, SEM_W2, SEM_X2 = range(8)
SEM_OUT = SEM_X0
NSEM = 8


def _pk(x):
    return pltpu.bitcast(x, U32)


def _upk(x):
    return pltpu.bitcast(x, BF16)


def _ln(x):
    m = jnp.mean(x, axis=-1, keepdims=True)
    xc = x - m
    v = jnp.mean(xc * xc, axis=-1, keepdims=True)
    return xc * lax.rsqrt(v + EPS)


def _ln_ln(x):
    m = jnp.mean(x, axis=-1, keepdims=True)
    xc = x - m
    v = jnp.mean(xc * xc, axis=-1, keepdims=True)
    return xc * lax.rsqrt(v * (1.0 + EPS) + EPS * EPS)


def _gelu(x):
    c0 = math.sqrt(2.0 / math.pi)
    c1 = c0 * 0.044715
    u = x * (c0 + c1 * (x * x))
    hx = 0.5 * x
    return hx + hx * jnp.tanh(u)


def _fold(op, xs):
    acc = xs[0]
    for x in xs[1:]:
        acc = op(acc, x)
    return acc


def _kernel(x_hbm, wqkv_hbm, wo_hbm, w1t_hbm, b1_hbm, w2_hbm, b2_hbm, out_hbm,
            xe, xo, wqkv_raw, wo_raw, w1t_s, b1_s, b2_s, wqkv_p, wo_p,
            qa, ka, va, qb, kb, vb, x1a, x1b, g_s, xn0_s, xn1_s, o_s, wo32, w1t_raw, w2_s, sems):
    step = pl.program_id(0)
    xbuf = (xe, xo)
    qs, ks, vs, x1s = (qa, qb), (ka, kb), (va, vb), (x1a, x1b)

    def rows_at(slot, r0, n):
        if isinstance(slot, int):
            return pl.ds(slot * T + r0, n)
        return pl.ds(pl.multiple_of(slot * T + r0, TH), n)

    def x_in_copy(t):
        sem = (SEM_X0, SEM_WV, SEM_W2, SEM_W2, SEM_X2, SEM_X2, SEM_X2, SEM_X2)[t]
        return pltpu.make_async_copy(
            x_hbm.at[0, pl.ds(t * T, T), :], xbuf[t % 2].at[pl.ds((t // 2) * T, T), :], sems.at[sem])

    def x_out_copy(par, slot, r0=0, n=T, c0=0, c1=D):
        return pltpu.make_async_copy(
            xbuf[par].at[rows_at(slot, r0, n), pl.ds(c0, c1 - c0)],
            out_hbm.at[0, rows_at(2 * slot + par, r0, n), pl.ds(c0, c1 - c0)],
            sems.at[SEM_OUT])

    def wqkv_copy(b, sem, r0=0, n=D):
        return pltpu.make_async_copy(
            wqkv_hbm.at[pl.ds(r0, n), pl.ds(b * D, D)], wqkv_raw.at[b, pl.ds(r0, n), :], sems.at[sem])

    def w1_group():
        return [pltpu.make_async_copy(wo_hbm, wo_raw, sems.at[SEM_W1]),
                pltpu.make_async_copy(w1t_hbm, w1t_raw, sems.at[SEM_W1]),
                pltpu.make_async_copy(b1_hbm, b1_s, sems.at[SEM_W1])]

    def w2_group():
        return [pltpu.make_async_copy(w2_hbm, w2_s, sems.at[SEM_W2]),
                pltpu.make_async_copy(b2_hbm, b2_s, sems.at[SEM_W2]),
                x_in_copy(2), x_in_copy(3)]

    def load_x(par, slot, r0=0, n=T):
        return xbuf[par][rows_at(slot, r0, n), :].astype(F32)

    def zoff(k):
        return pl.multiple_of(lax.shift_right_logical(step, k) * 8, 8)

    def proj(xn, par, c0, c1, r0=0, n=T):
        qscale = (DH ** -0.5) * LOG2E
        res = jnp.dot(xn, _upk(wqkv_p[:, c0:c1]), preferred_element_type=F32)
        for c in range(c0, c1, 128):
            blk = res[:, c - c0:c - c0 + 128]
            b, j = c // D, (c % D) // 128
            if b == 0:
                qs[par][r0:r0 + n, j * 128:(j + 1) * 128] = blk * qscale
            elif b == 1:
                ks[par][j, HALO + r0:HALO + r0 + n, :] = blk
            else:
                vs[par][j, HALO + r0:HALO + r0 + n, :] = blk

    def halo_copy(par):
        for j in range(NL):
            ks[par][j, 0:HALO, :] = ks[1 - par][j, T:T + HALO, :]
            vs[par][j, 0:HALO, :] = vs[1 - par][j, T:T + HALO, :]

    def attention(par, row0, chain, ra=0, rb=T, hooks=None):
        q_s, k_s, v_s = qs[par], ks[par], vs[par]
        chunks = list(range(ra // R, rb // R))
        z1, z2 = zoff(10), zoff(11)

        def load_q(c):
            qq = q_s[pl.ds(z1 + c * R, R), :]
            return [qq[:, j * 128:(j + 1) * 128] for j in range(NL)]

        pend = {c: load_q(c) for c in chunks[:chain]}
        for c in chunks:
            r0 = c * R
            q = pend.pop(c)
            logits = []
            for w in range(W):
                st = HALO + r0 - DIL * w
                acc = _fold(jnp.add, [q[j] * k_s[j, st:st + R, :] for j in range(NL)])
                acc = acc + pltpu.roll(acc, 64, 1)
                acc = acc + pltpu.roll(acc, 32, 1)
                if r0 < DIL * w:
                    row = lax.broadcasted_iota(jnp.int32, (R, 128), 0) + (row0 + r0)
                    acc = jnp.where(row >= DIL * w, acc, -1e9 * LOG2E)
                logits.append(acc)
            m = _fold(jnp.maximum, logits)
            ps = [jnp.exp2(lg - m) for lg in logits]
            inv = pl.reciprocal(_fold(jnp.add, ps), approx=True)
            outs = []
            for j in range(NL):
                acc = _fold(jnp.add, [ps[w] * v_s[j, HALO + r0 - DIL * w:HALO + r0 - DIL * w + R, :]
                                      for w in range(W)])
                outs.append(acc * inv)
            o_s[r0:r0 + R, :] = jnp.concatenate(outs, axis=1)
            q_s[pl.ds(z2 + T, 8), 0:128] = outs[1]
            if c + chain <= chunks[-1]:
                pend[c + chain] = load_q(c + chain)
            if hooks and (r0 + R) in hooks:
                hooks[r0 + R](outs[NL - 1])

    def w2_part(par, slot, c0, c1, r0=0, n=T, g=None):
        if g is None:
            g = _upk(g_s[r0 // 2:(r0 + n) // 2, :])
        b2 = b2_s[...].astype(F32)[None, :]
        acc = jnp.dot(g, w2_s[:, c0:c1], preferred_element_type=F32)
        x2 = x1s[par][r0:r0 + n, c0:c1] + (acc + b2[:, c0:c1])
        xbuf[par][rows_at(slot, r0, n), c0:c1] = x2.astype(BF16)

    def wo_mm(par, slot, r0=0, n=T):
        o = o_s[r0:r0 + n, :].astype(BF16)
        x1 = load_x(par, slot, r0, n) + jnp.dot(o, _upk(wo_p[...]), preferred_element_type=F32)
        x1s[par][r0:r0 + n, :] = x1
        return x1

    def ln2_after(par, r0, n, tok):
        x1s[par][pl.ds(zoff(11) + T, 8), 0:128] = tok
        return _ln_ln(x1s[par][pl.ds(zoff(10) + r0, n), :]).astype(BF16)

    def wo_ln2(par, slot, r0=0, n=T):
        return _ln_ln(wo_mm(par, slot, r0, n)).astype(BF16)

    def w1_gelu(y, r0=0, n=T):
        b1 = b1_s[...].astype(F32)[None, :]
        h = lax.dot_general(y, _upk(w1t_s[...]), NT_DIMS, preferred_element_type=F32) + b1
        gl = _gelu(h)
        g_s[r0 // 2:(r0 + n) // 2, :] = _pk(gl.astype(BF16))
        return gl

    def slot_body(sig, par, pace_next):
        slot_b = (sig % NT) // 2
        slot_c = ((sig + NT - 1) % NT) // 2
        slot_a = ((sig + 1) % NT) // 2
        xa = load_x(1 - par, slot_a)
        g = _upk(g_s[...])
        w2_part(1 - par, slot_c, 0, NSPLIT, g=g)
        proj(_ln(xa).astype(BF16), 1 - par, 0, 3 * D)
        halo_copy(1 - par)
        attention(par, (sig % NT) * T, CHAIN)
        y = wo_ln2(par, slot_b)
        w2_part(1 - par, slot_c, NSPLIT, D, g=g)
        gl = w1_gelu(y)
        if pace_next:
            tok = gl[T - 16:T, F - 96:F]
            qs[1 - par][pl.ds(zoff(11) + T, 8), 0:96] = tok[8:16]
            xbuf[par][pl.ds(pl.multiple_of(zoff(11) * 2 + S // 2, 16), 16), 0:96] = tok.astype(BF16)

    def prep_qkv(b, r0=0, n=D):
        w = _pk(wqkv_raw[b, r0:r0 + n, :])
        lane = lax.broadcasted_iota(jnp.int32, (n // 2, 128), 1)
        a_src = (lane // 4) % 4
        for j in range(NL):
            acc = w[:, 0:128]
            for J in range(1, NL):
                acc = jnp.where(a_src == (j + J) % 4, w[:, J * 128:(J + 1) * 128], acc)
            idx = (lane % 8) * 16 + 4 * ((lane // 8 + j) % 4) + lane // 32
            wqkv_p[r0 // 2:(r0 + n) // 2, b * D + j * 128:b * D + (j + 1) * 128] = (
                jnp.take_along_axis(acc, idx, axis=1))

    def prep_wo():
        lo = jnp.uint32(0xFFFF)
        hi = jnp.uint32(0xFFFF0000)
        grp = lax.broadcasted_iota(jnp.int32, (16, 128), 0) // 4
        for c in range(NL):
            wo32[c] = _pk(wo_raw[:, c * 128:(c + 1) * 128])
            src32 = wo32.at[c]
            blk = []
            for t in range(DH // 2):
                ev = src32[pl.ds(t, 16, stride=16), :]
                od = src32[pl.ds(8 + t, 16, stride=16), :]
                blk.append((ev & lo) | (od << 16))
                blk.append((ev >> 16) | (od & hi))
            for j in range(NL):
                for e in range(4):
                    acc = blk[4 * j + e]
                    for J in range(1, NL):
                        acc = jnp.where(grp == J, blk[4 * ((j + J) % 4) + e], acc)
                    wo_p[j * 64 + e * 16:j * 64 + (e + 1) * 16, c * 128:(c + 1) * 128] = acc

    @pl.when(step == 0)
    def _first():
        wq0 = wqkv_copy(0, SEM_WQ0, 0, D // 2)
        wq1 = wqkv_copy(0, SEM_WQ1, D // 2, D // 2)
        wk = wqkv_copy(1, SEM_WK)
        wv = wqkv_copy(2, SEM_WV)
        for c in ([x_in_copy(0), wq0, wq1, wk, wv, x_in_copy(1)] + w1_group() + w2_group()
                  + [x_in_copy(t) for t in range(4, NT)]):
            c.start()
        z = jnp.zeros((HALO, 128), F32)
        for j in range(NL):
            ka[j, 0:HALO, :] = z
            va[j, 0:HALO, :] = z
        x_in_copy(0).wait()
        xn0_s[...] = _pk(_ln(load_x(0, 0)).astype(BF16))
        wq0.wait()
        prep_qkv(0, 0, D // 2)
        wq1.wait()
        prep_qkv(0, D // 2, D // 2)
        proj(_upk(xn0_s[...]), 0, 0, QS)
        wk.wait()
        prep_qkv(1)
        proj(_upk(xn0_s[...]), 0, QS, KS)
        wv.wait()
        x_in_copy(1).wait()
        prep_qkv(2)
        proj(_upk(xn0_s[...]), 0, KS, 2 * D)
        proj(_upk(xn0_s[0:TH // 2, :]), 0, 2 * D, 3 * D, 0, TH)
        proj(_upk(xn0_s[TH // 2:T // 2, :]), 0, 2 * D, 3 * D, TH, TH)
        xn1 = _ln(load_x(1, 0)).astype(BF16)
        xn1_s[...] = _pk(xn1)
        proj(xn1, 1, 0, V0)
        attention(0, 0, CHAIN, 0, RA)
        for c in w1_group():
            c.wait()
        prep_wo()
        w1t_s[...] = _pk(w1t_raw[...])
        proj(_upk(xn1_s[...]), 1, V0, 3 * D)
        halo_copy(1)
        wo_mm(0, 0, 0, TH)
        ys = []
        attention(0, 0, 2 * CHAIN, RA, T, hooks={T: lambda tok: ys.append(ln2_after(0, 0, TH, tok))})
        yb = wo_ln2(0, 0, TH, TH)
        w1_gelu(ys[0], 0, TH)
        w1_gelu(yb, TH, TH)
        for c in w2_group():
            c.wait()

    @pl.when(step == 2)
    def _():
        for t in range(4, NT):
            x_in_copy(t).wait()

    @pl.when(jnp.logical_and(step > 0, step < NSTEPS - 1))
    def _mid():
        for _slot in range(NT // 2 - 2):
            @pl.when(step == NT // 2 + 2 + _slot)
            def _(slot=_slot):
                x_out_copy(0, slot).start()
                x_out_copy(1, slot).start()

        slot_body(2 * step - 1, 1, True)
        slot_body(2 * step, 0, False)

    @pl.when(step == NSTEPS - 1)
    def _last():
        sl = NT // 2 - 1
        x_out_copy(0, sl - 1).start()
        x_out_copy(1, sl - 1).start()
        g = _upk(g_s[...])
        w2_part(0, sl, 0, NSPLIT, g=g)
        ys = []
        attention(1, (NT - 1) * T, CHAIN, 0, T,
                  hooks={TH: lambda tok: wo_mm(1, sl, 0, TH),
                         HKL: lambda tok: ys.append(ln2_after(1, 0, TH, tok))})
        w2_part(0, sl, NSPLIT, D, g=g)
        w1_gelu(ys[0], 0, TH)
        yb = wo_ln2(1, sl, TH, TH)
        w2_part(1, sl, 0, D, 0, TH)
        w1_gelu(yb, TH, TH)
        tail = [x_out_copy(0, sl), x_out_copy(1, sl, 0, TH),
                x_out_copy(1, sl, TH, TH, 0, LS), x_out_copy(1, sl, TH, TH, LS, D)]
        tail[0].start()
        tail[1].start()
        w2_part(1, sl, 0, LS, TH, TH)
        tail[2].start()
        w2_part(1, sl, LS, D, TH, TH)
        tail[3].start()
        for t in range(NT - 2):
            x_out_copy(t % 2, t // 2).wait()
        for c in tail:
            c.wait()


@jax.jit
def pallas_interleave_layers__sliding_local_dilated__mixer_channel_mlp__prompt_kernel(
    A_x: jax.Array,
    A_wqkv: jax.Array,
    A_wo: jax.Array,
    B_x: jax.Array,
    B_w1: jax.Array,
    B_b1: jax.Array,
    B_w2: jax.Array,
    B_b2: jax.Array,
):
    del B_x
    any_spec = pl.BlockSpec(memory_space=pl.ANY)
    kv = pltpu.VMEM((NL, HALO + T, 128), F32)
    tq = pltpu.VMEM((T + 8, D), F32)
    return pl.pallas_call(
        _kernel,
        grid=(NSTEPS,),
        in_specs=[any_spec] * 7,
        out_specs=any_spec,
        out_shape=jax.ShapeDtypeStruct((1, S, D), A_x.dtype),
        scratch_shapes=[
            pltpu.VMEM((S // 2 + 16, D), BF16),
            pltpu.VMEM((S // 2 + 16, D), BF16),
            pltpu.VMEM((3, D, D), BF16),
            pltpu.VMEM((D, D), BF16),
            pltpu.VMEM((F // 2, D), U32),
            pltpu.VMEM((F,), BF16),
            pltpu.VMEM((D,), BF16),
            pltpu.VMEM((D // 2, 3 * D), U32),
            pltpu.VMEM((D // 2, D), U32),
            tq, kv, kv, tq, kv, kv,
            tq, tq,
            pltpu.VMEM((T // 2, F), U32),
            pltpu.VMEM((T // 2, D), U32),
            pltpu.VMEM((T // 2, D), U32),
            pltpu.VMEM((T, D), F32),
            pltpu.VMEM((NL, D // 2, 128), U32),
            pltpu.VMEM((F, D), BF16),
            pltpu.VMEM((F, D), BF16),
            pltpu.SemaphoreType.DMA((NSEM,)),
        ],
        compiler_params=pltpu.CompilerParams(
            dimension_semantics=("arbitrary",),
            vmem_limit_bytes=64 * 1024 * 1024,
        ),
    )(A_x, A_wqkv, A_wo, B_w1.T, B_b1, B_w2, B_b2)
```

```python
import math

import jax
import jax.numpy as jnp
from jax import lax
import jax.experimental.pallas as pl
import jax.experimental.pallas.tpu as pltpu

S, D, F = 2048, 512, 1376
H, DH, W, DIL = 32, 16, 8, 2
EPS = 1e-5

T = 256
TH = T // 2
R = 8
HALO = 16
NL = D // 128
NT = S // T
NITEMS = 2 * NT
NSTEPS = NITEMS // 2 + 1
FM = (F // 128) * 128

NSPLIT = 384
CHAIN = 3
QS, KS, V0, RA = 256, 896, 1408, 208
HKL = 168
HT = 512
LS = 256

F32 = jnp.float32
BF16 = jnp.bfloat16
U32 = jnp.uint32
NT_DIMS = (((1,), (1,)), ((), ()))
LOG2E = math.log2(math.e)

SEM_X0, SEM_WQ0, SEM_WQ1, SEM_WK, SEM_WV, SEM_W1, SEM_W2, SEM_X2 = range(8)
SEM_OUT = SEM_X0
NSEM = 8


def _pk(x):
    return pltpu.bitcast(x, U32)


def _upk(x):
    return pltpu.bitcast(x, BF16)


def _ln(x):
    m = jnp.mean(x, axis=-1, keepdims=True)
    xc = x - m
    v = jnp.mean(xc * xc, axis=-1, keepdims=True)
    return xc * lax.rsqrt(v + EPS)


def _ln_ln(x):
    m = jnp.mean(x, axis=-1, keepdims=True)
    xc = x - m
    v = jnp.mean(xc * xc, axis=-1, keepdims=True)
    return xc * lax.rsqrt(v * (1.0 + EPS) + EPS * EPS)


def _gelu(x):
    c0 = math.sqrt(2.0 / math.pi)
    c1 = c0 * 0.044715
    u = x * (c0 + c1 * (x * x))
    hx = 0.5 * x
    return hx + hx * jnp.tanh(u)


def _fold(op, xs):
    acc = xs[0]
    for x in xs[1:]:
        acc = op(acc, x)
    return acc


def _kernel(x_hbm, wqkv_hbm, wo_hbm, w1t_hbm, b1_hbm, w2_hbm, b2_hbm, out_hbm,
            xe, xo, wqkv_raw, wo_raw, w1t_s, b1_s, b2_s, wqkv_p, wo_p,
            qa, ka, va, qb, kb, vb, x1a, x1b, g_s, xn0_s, xn1_s, o_s, wo32, w1t_raw, w2_s, sems):
    step = pl.program_id(0)
    xbuf = (xe, xo)
    qs, ks, vs, x1s = (qa, qb), (ka, kb), (va, vb), (x1a, x1b)

    def rows_at(slot, r0, n):
        if isinstance(slot, int):
            return pl.ds(slot * T + r0, n)
        return pl.ds(pl.multiple_of(slot * T + r0, TH), n)

    def x_in_copy(t):
        sem = (SEM_X0, SEM_WV, SEM_W2, SEM_W2, SEM_X2, SEM_X2, SEM_X2, SEM_X2)[t]
        return pltpu.make_async_copy(
            x_hbm.at[0, pl.ds(t * T, T), :], xbuf[t % 2].at[pl.ds((t // 2) * T, T), :], sems.at[sem])

    def x_out_copy(par, slot, r0=0, n=T, c0=0, c1=D):
        return pltpu.make_async_copy(
            xbuf[par].at[rows_at(slot, r0, n), pl.ds(c0, c1 - c0)],
            out_hbm.at[0, rows_at(2 * slot + par, r0, n), pl.ds(c0, c1 - c0)],
            sems.at[SEM_OUT])

    def wqkv_copy(b, sem, r0=0, n=D):
        return pltpu.make_async_copy(
            wqkv_hbm.at[pl.ds(r0, n), pl.ds(b * D, D)], wqkv_raw.at[b, pl.ds(r0, n), :], sems.at[sem])

    def w1_group():
        return [pltpu.make_async_copy(wo_hbm, wo_raw, sems.at[SEM_W1]),
                pltpu.make_async_copy(w1t_hbm, w1t_raw, sems.at[SEM_W1]),
                pltpu.make_async_copy(b1_hbm, b1_s, sems.at[SEM_W1])]

    def w2_group():
        return [pltpu.make_async_copy(w2_hbm, w2_s, sems.at[SEM_W2]),
                pltpu.make_async_copy(b2_hbm, b2_s, sems.at[SEM_W2]),
                x_in_copy(2), x_in_copy(3)]

    def load_x(par, slot, r0=0, n=T):
        return xbuf[par][rows_at(slot, r0, n), :].astype(F32)

    def zoff(k):
        return pl.multiple_of(lax.shift_right_logical(step, k) * 8, 8)

    def proj(xn, par, c0, c1, r0=0, n=T):
        qscale = (DH ** -0.5) * LOG2E
        res = jnp.dot(xn, _upk(wqkv_p[:, c0:c1]), preferred_element_type=F32)
        for c in range(c0, c1, 128):
            blk = res[:, c - c0:c - c0 + 128]
            b, j = c // D, (c % D) // 128
            if b == 0:
                qs[par][r0:r0 + n, j * 128:(j + 1) * 128] = blk * qscale
            elif b == 1:
                ks[par][j, HALO + r0:HALO + r0 + n, :] = blk
            else:
                vs[par][j, HALO + r0:HALO + r0 + n, :] = blk

    def halo_copy(par):
        for j in range(NL):
            ks[par][j, 0:HALO, :] = ks[1 - par][j, T:T + HALO, :]
            vs[par][j, 0:HALO, :] = vs[1 - par][j, T:T + HALO, :]

    def attention(par, row0, chain, ra=0, rb=T, hooks=None):
        q_s, k_s, v_s = qs[par], ks[par], vs[par]
        chunks = list(range(ra // R, rb // R))
        z1, z2 = zoff(10), zoff(11)

        def load_q(c):
            qq = q_s[pl.ds(z1 + c * R, R), :]
            return [qq[:, j * 128:(j + 1) * 128] for j in range(NL)]

        pend = {c: load_q(c) for c in chunks[:chain]}
        for c in chunks:
            r0 = c * R
            q = pend.pop(c)
            logits = []
            for w in range(W):
                st = HALO + r0 - DIL * w
                acc = _fold(jnp.add, [q[j] * k_s[j, st:st + R, :] for j in range(NL)])
                acc = acc + pltpu.roll(acc, 64, 1)
                acc = acc + pltpu.roll(acc, 32, 1)
                if r0 < DIL * w:
                    row = lax.broadcasted_iota(jnp.int32, (R, 128), 0) + (row0 + r0)
                    acc = jnp.where(row >= DIL * w, acc, -1e9 * LOG2E)
                logits.append(acc)
            m = _fold(jnp.maximum, logits)
            ps = [jnp.exp2(lg - m) for lg in logits]
            inv = pl.reciprocal(_fold(jnp.add, ps), approx=True)
            outs = []
            for j in range(NL):
                acc = _fold(jnp.add, [ps[w] * v_s[j, HALO + r0 - DIL * w:HALO + r0 - DIL * w + R, :]
                                      for w in range(W)])
                outs.append(acc * inv)
            o_s[r0:r0 + R, :] = jnp.concatenate(outs, axis=1)
            q_s[pl.ds(z2 + T, 8), 0:128] = outs[1]
            if c + chain <= chunks[-1]:
                pend[c + chain] = load_q(c + chain)
            if hooks and (r0 + R) in hooks:
                hooks[r0 + R](outs[NL - 1])

    def w2_part(par, slot, c0, c1, r0=0, n=T, g=None):
        if g is None:
            g = _upk(g_s[r0 // 2:(r0 + n) // 2, :])
        b2 = b2_s[...].astype(F32)[None, :]
        acc = jnp.dot(g, w2_s[:, c0:c1], preferred_element_type=F32)
        x2 = x1s[par][r0:r0 + n, c0:c1] + (acc + b2[:, c0:c1])
        xbuf[par][rows_at(slot, r0, n), c0:c1] = x2.astype(BF16)

    def wo_mm(par, slot, r0=0, n=T):
        o = o_s[r0:r0 + n, :].astype(BF16)
        x1 = load_x(par, slot, r0, n) + jnp.dot(o, _upk(wo_p[...]), preferred_element_type=F32)
        x1s[par][r0:r0 + n, :] = x1
        return x1

    def ln2_after(par, r0, n, tok):
        x1s[par][pl.ds(zoff(11) + T, 8), 0:128] = tok
        return _ln_ln(x1s[par][pl.ds(zoff(10) + r0, n), :]).astype(BF16)

    def wo_ln2(par, slot, r0=0, n=T):
        return _ln_ln(wo_mm(par, slot, r0, n)).astype(BF16)

    def w1_gelu(y, r0=0, n=T):
        b1 = b1_s[...].astype(F32)[None, :]
        h0 = lax.dot_general(y, _upk(w1t_s[0:HT // 2, :]), NT_DIMS, preferred_element_type=F32)
        ht = lax.dot_general(_upk(w1t_s[FM // 2:F // 2, :]), y, NT_DIMS, preferred_element_type=F32)
        h1 = lax.dot_general(y, _upk(w1t_s[HT // 2:FM // 2, :]), NT_DIMS, preferred_element_type=F32)
        h = jnp.concatenate([h0, h1, ht.T], axis=1) + b1
        gl = _gelu(h)
        g_s[r0 // 2:(r0 + n) // 2, :] = _pk(gl.astype(BF16))
        return gl

    def slot_body(sig, par, pace_next):
        slot_b = (sig % NT) // 2
        slot_c = ((sig + NT - 1) % NT) // 2
        slot_a = ((sig + 1) % NT) // 2
        xa = load_x(1 - par, slot_a)
        g = _upk(g_s[...])
        w2_part(1 - par, slot_c, 0, NSPLIT, g=g)
        proj(_ln(xa).astype(BF16), 1 - par, 0, 3 * D)
        halo_copy(1 - par)
        attention(par, (sig % NT) * T, CHAIN)
        y = wo_ln2(par, slot_b)
        w2_part(1 - par, slot_c, NSPLIT, D, g=g)
        gl = w1_gelu(y)
        if pace_next:
            tok = gl[T - 16:T, FM - 128:FM]
            qs[1 - par][pl.ds(zoff(11) + T, 8), 0:128] = tok[8:16]
            xbuf[par][pl.ds(pl.multiple_of(zoff(11) * 2 + S // 2, 16), 16), 0:128] = tok.astype(BF16)

    def prep_qkv(b, r0=0, n=D):
        w = _pk(wqkv_raw[b, r0:r0 + n, :])
        lane = lax.broadcasted_iota(jnp.int32, (n // 2, 128), 1)
        a_src = (lane // 4) % 4
        for j in range(NL):
            acc = w[:, 0:128]
            for J in range(1, NL):
                acc = jnp.where(a_src == (j + J) % 4, w[:, J * 128:(J + 1) * 128], acc)
            idx = (lane % 8) * 16 + 4 * ((lane // 8 + j) % 4) + lane // 32
            wqkv_p[r0 // 2:(r0 + n) // 2, b * D + j * 128:b * D + (j + 1) * 128] = (
                jnp.take_along_axis(acc, idx, axis=1))

    def prep_wo():
        lo = jnp.uint32(0xFFFF)
        hi = jnp.uint32(0xFFFF0000)
        grp = lax.broadcasted_iota(jnp.int32, (16, 128), 0) // 4
        for c in range(NL):
            wo32[c] = _pk(wo_raw[:, c * 128:(c + 1) * 128])
            src32 = wo32.at[c]
            blk = []
            for t in range(DH // 2):
                ev = src32[pl.ds(t, 16, stride=16), :]
                od = src32[pl.ds(8 + t, 16, stride=16), :]
                blk.append((ev & lo) | (od << 16))
                blk.append((ev >> 16) | (od & hi))
            for j in range(NL):
                for e in range(4):
                    acc = blk[4 * j + e]
                    for J in range(1, NL):
                        acc = jnp.where(grp == J, blk[4 * ((j + J) % 4) + e], acc)
                    wo_p[j * 64 + e * 16:j * 64 + (e + 1) * 16, c * 128:(c + 1) * 128] = acc

    @pl.when(step == 0)
    def _first():
        wq0 = wqkv_copy(0, SEM_WQ0, 0, D // 2)
        wq1 = wqkv_copy(0, SEM_WQ1, D // 2, D // 2)
        wk = wqkv_copy(1, SEM_WK)
        wv = wqkv_copy(2, SEM_WV)
        for c in ([x_in_copy(0), wq0, wq1, wk, wv, x_in_copy(1)] + w1_group() + w2_group()
                  + [x_in_copy(t) for t in range(4, NT)]):
            c.start()
        z = jnp.zeros((HALO, 128), F32)
        for j in range(NL):
            ka[j, 0:HALO, :] = z
            va[j, 0:HALO, :] = z
        x_in_copy(0).wait()
        xn0_s[...] = _pk(_ln(load_x(0, 0)).astype(BF16))
        wq0.wait()
        prep_qkv(0, 0, D // 2)
        wq1.wait()
        prep_qkv(0, D // 2, D // 2)
        proj(_upk(xn0_s[...]), 0, 0, QS)
        wk.wait()
        prep_qkv(1)
        proj(_upk(xn0_s[...]), 0, QS, KS)
        wv.wait()
        x_in_copy(1).wait()
        prep_qkv(2)
        proj(_upk(xn0_s[...]), 0, KS, 2 * D)
        proj(_upk(xn0_s[0:TH // 2, :]), 0, 2 * D, 3 * D, 0, TH)
        proj(_upk(xn0_s[TH // 2:T // 2, :]), 0, 2 * D, 3 * D, TH, TH)
        xn1 = _ln(load_x(1, 0)).astype(BF16)
        xn1_s[...] = _pk(xn1)
        proj(xn1, 1, 0, V0)
        attention(0, 0, CHAIN, 0, RA)
        for c in w1_group():
            c.wait()
        prep_wo()
        w1t_s[...] = _pk(w1t_raw[...])
        proj(_upk(xn1_s[...]), 1, V0, 3 * D)
        halo_copy(1)
        wo_mm(0, 0, 0, TH)
        ys = []
        attention(0, 0, 2 * CHAIN, RA, T, hooks={T: lambda tok: ys.append(ln2_after(0, 0, TH, tok))})
        yb = wo_ln2(0, 0, TH, TH)
        w1_gelu(ys[0], 0, TH)
        w1_gelu(yb, TH, TH)
        for c in w2_group():
            c.wait()

    @pl.when(step == 2)
    def _():
        for t in range(4, NT):
            x_in_copy(t).wait()

    @pl.when(jnp.logical_and(step > 0, step < NSTEPS - 1))
    def _mid():
        for _slot in range(NT // 2 - 2):
            @pl.when(step == NT // 2 + 2 + _slot)
            def _(slot=_slot):
                x_out_copy(0, slot).start()
                x_out_copy(1, slot).start()

        slot_body(2 * step - 1, 1, True)
        slot_body(2 * step, 0, False)

    @pl.when(step == NSTEPS - 1)
    def _last():
        sl = NT // 2 - 1
        x_out_copy(0, sl - 1).start()
        x_out_copy(1, sl - 1).start()
        g = _upk(g_s[...])
        w2_part(0, sl, 0, NSPLIT, g=g)
        ys = []
        attention(1, (NT - 1) * T, CHAIN, 0, T,
                  hooks={TH: lambda tok: wo_mm(1, sl, 0, TH),
                         HKL: lambda tok: ys.append(ln2_after(1, 0, TH, tok))})
        w2_part(0, sl, NSPLIT, D, g=g)
        w1_gelu(ys[0], 0, TH)
        yb = wo_ln2(1, sl, TH, TH)
        w2_part(1, sl, 0, D, 0, TH)
        w1_gelu(yb, TH, TH)
        tail = [x_out_copy(0, sl), x_out_copy(1, sl, 0, TH),
                x_out_copy(1, sl, TH, TH, 0, LS), x_out_copy(1, sl, TH, TH, LS, D)]
        tail[0].start()
        tail[1].start()
        w2_part(1, sl, 0, LS, TH, TH)
        tail[2].start()
        w2_part(1, sl, LS, D, TH, TH)
        tail[3].start()
        for t in range(NT - 2):
            x_out_copy(t % 2, t // 2).wait()
        for c in tail:
            c.wait()


@jax.jit
def pallas_interleave_layers__sliding_local_dilated__mixer_channel_mlp__prompt_kernel(
    A_x: jax.Array,
    A_wqkv: jax.Array,
    A_wo: jax.Array,
    B_x: jax.Array,
    B_w1: jax.Array,
    B_b1: jax.Array,
    B_w2: jax.Array,
    B_b2: jax.Array,
):
    del B_x
    any_spec = pl.BlockSpec(memory_space=pl.ANY)
    kv = pltpu.VMEM((NL, HALO + T, 128), F32)
    tq = pltpu.VMEM((T + 8, D), F32)
    return pl.pallas_call(
        _kernel,
        grid=(NSTEPS,),
        in_specs=[any_spec] * 7,
        out_specs=any_spec,
        out_shape=jax.ShapeDtypeStruct((1, S, D), A_x.dtype),
        scratch_shapes=[
            pltpu.VMEM((S // 2 + 16, D), BF16),
            pltpu.VMEM((S // 2 + 16, D), BF16),
            pltpu.VMEM((3, D, D), BF16),
            pltpu.VMEM((D, D), BF16),
            pltpu.VMEM((F // 2, D), U32),
            pltpu.VMEM((F,), BF16),
            pltpu.VMEM((D,), BF16),
            pltpu.VMEM((D // 2, 3 * D), U32),
            pltpu.VMEM((D // 2, D), U32),
            tq, kv, kv, tq, kv, kv,
            tq, tq,
            pltpu.VMEM((T // 2, F), U32),
            pltpu.VMEM((T // 2, D), U32),
            pltpu.VMEM((T // 2, D), U32),
            pltpu.VMEM((T, D), F32),
            pltpu.VMEM((NL, D // 2, 128), U32),
            pltpu.VMEM((F, D), BF16),
            pltpu.VMEM((F, D), BF16),
            pltpu.SemaphoreType.DMA((NSEM,)),
        ],
        compiler_params=pltpu.CompilerParams(
            dimension_semantics=("arbitrary",),
            vmem_limit_bytes=64 * 1024 * 1024,
        ),
    )(A_x, A_wqkv, A_wo, B_w1.T, B_b1, B_w2, B_b2)
```
